```python
import jax
import jax.numpy as jnp

def _softmax(x, axis=-1):
    return jax.nn.softmax(x, axis=axis)
def _gelu(x):
    return jax.nn.gelu(x, approximate=True)
def _silu(x):
    return jax.nn.silu(x)
def _sigmoid(x):
    return jax.nn.sigmoid(x)
def _layernorm(x, axis=-1, eps=1e-5):
    m = jnp.mean(x, axis=axis, keepdims=True)
    v = jnp.var(x, axis=axis, keepdims=True)
    return (x - m) / jnp.sqrt(v + eps)
def _scatter_add(tgt, idx, src, axis=0):
    return tgt.at[idx].add(src)
def _segment_sum(src, seg, n):
    return jax.ops.segment_sum(src, seg, n)
class _Rng:
    def __init__(self, key):
        self._k = key
    def _next(self):
        self._k, sub = jax.random.split(self._k)
        return sub
    def normal(self, shape):
        return jax.random.normal(self._next(), shape, dtype=jnp.bfloat16)
    def randint(self, lo, hi, shape):
        return jax.random.randint(self._next(), shape, lo, hi, dtype=jnp.int32)
    def uniform(self, shape, lo=0.0, hi=1.0):
        return jax.random.uniform(self._next(), shape, jnp.bfloat16, lo, hi)
    def permutation(self, n):
        return jax.random.permutation(self._next(), n)


kernel_name = 'sequential_preLN__sliding_block_cached__glu_gated_swiglu__decode'

def setup_inputs():
    _rng = _Rng(jax.random.key(int.from_bytes(__import__("os").urandom(4), "little")))
    _w = (lambda a: (lambda t: t.astype(jnp.bfloat16) if jnp.issubdtype(t.dtype, jnp.floating) else t)(jnp.asarray(a)))
    def _A_setup():
        B, Sq, D = 1, 1, 640
        Hq, Hkv, Sk, Dh = 32, 32, 32768, 192
        assert Hq % Hkv == 0, (Hq, Hkv)
        return {
            "x": _w((lambda *s: _rng.normal(s) * 0.05)(B, Sq, D)),
            "k_cache": _w((lambda *s: _rng.normal(s) * 0.05)(B, Hkv, Sk, Dh)),
            "v_cache": _w((lambda *s: _rng.normal(s) * 0.05)(B, Hkv, Sk, Dh)),
            "wq": _w((lambda *s: _rng.normal(s) * 0.05)(D, Hq * Dh) * (D ** -0.5)),
            "wo": _w((lambda *s: _rng.normal(s) * 0.05)(Hq * Dh, D) * ((Hq * Dh) ** -0.5)),
        }
    _A_in = _A_setup()

    def _B_setup():
        B, S, D, F = 1, 1, 640, 1536
        return {
            "x": _w((lambda *s: _rng.normal(s) * 0.05)(B, S, D)),
            "w1": _w((lambda *s: _rng.normal(s) * 0.05)(D, F) * (2.0 / D) ** 0.5),
            "w3": _w((lambda *s: _rng.normal(s) * 0.05)(D, F) * (2.0 / D) ** 0.5),
            "w2": _w((lambda *s: _rng.normal(s) * 0.05)(F, D) * (2.0 / F) ** 0.5),
        }
    _B_in = _B_setup()

    return {
        "A_x": _A_in["x"],
        "A_k_cache": _A_in["k_cache"],
        "A_v_cache": _A_in["v_cache"],
        "A_wq": _A_in["wq"],
        "A_wo": _A_in["wo"],
        "B_x": _B_in["x"],
        "B_w1": _B_in["w1"],
        "B_w3": _B_in["w3"],
        "B_w2": _B_in["w2"],
    }

def reference(A_x, A_k_cache, A_v_cache, A_wq, A_wo, B_x, B_w1, B_w3, B_w2):
    def _A_ref(x, k_cache, v_cache, wq, wo):
        B, Sq, D = x.shape
        Hq, Dh = 32, 192
        Hkv, Sk = k_cache.shape[1], k_cache.shape[2]
        W = min(4096, max(256, Sk // 4))
        rep = Hq // Hkv
        q = (lambda x, *d: x.transpose(*d))((x @ wq).reshape(B, Sq, Hq, Dh), 0, 2, 1, 3)
        k = jnp.repeat(k_cache[:, :, Sk - W:, :], rep, axis=1)
        v = jnp.repeat(v_cache[:, :, Sk - W:, :], rep, axis=1)
        scores = jnp.einsum("bhqd,bhkd->bhqk", q, k) * (Dh ** -0.5)
        p = _softmax(scores, axis=-1)
        o = jnp.einsum("bhqk,bhkd->bhqd", p, v)
        return (lambda x, *d: x.transpose(*d))(o, 0, 2, 1, 3).reshape(B, Sq, Hq * Dh) @ wo

    def _B_ref(x, w1, w3, w2):
        gate = jnp.einsum("bsd,df->bsf", x, w1)
        up = jnp.einsum("bsd,df->bsf", x, w3)
        h = _silu(gate) * up
        out = jnp.einsum("bsf,fd->bsd", h, w2)
        return out

    x = A_x
    h = x + _A_ref(_layernorm(x, axis=-1), A_k_cache, A_v_cache, A_wq, A_wo)
    h2 = h + _B_ref(_layernorm(h, axis=-1), B_w1, B_w3, B_w2)
    return h2
```

```python
import functools
import jax
import jax.numpy as jnp
import numpy as np
import jax.experimental.pallas as pl
import jax.experimental.pallas.tpu as pltpu

D = 640
H = 32
DH = 192
SK = 32768
W = 4096
F = 1536
EPS = 1e-5


def _ln(x):
    m = jnp.mean(x, axis=-1, keepdims=True)
    xc = x - m
    v = jnp.mean(xc * xc, axis=-1, keepdims=True)
    return xc * jax.lax.rsqrt(v + EPS)


def make_kernel(NSLOT=4, WO_CH=4, W2_SPLIT=1280):
    NPAIR = H // 2
    assert NSLOT % 2 == 0
    PSL = NSLOT // 2

    def kernel(x_hbm, k_hbm, v_hbm, wq_hbm, wo_hbm, w1_hbm, w3_hbm, w2_hbm, o_ref,
               x_buf, wq_buf, wo_buf, w1_buf, w3_buf, w2_buf, k_buf, v_buf, q_scr, o_scr,
               sem_misc, sem_k, sem_v):
        x_cp = pltpu.make_async_copy(x_hbm.at[0], x_buf, sem_misc.at[0])
        wq_cp = pltpu.make_async_copy(wq_hbm, wq_buf, sem_misc.at[1])
        wo_rows = (H * DH) // WO_CH
        wo_cps = [pltpu.make_async_copy(wo_hbm.at[pl.ds(i * wo_rows, wo_rows), :],
                                        wo_buf.at[pl.ds(i * wo_rows, wo_rows), :], sem_misc.at[2 + i])
                  for i in range(WO_CH)]
        w1_cp = pltpu.make_async_copy(w1_hbm, w1_buf, sem_misc.at[2 + WO_CH])
        w3_cp = pltpu.make_async_copy(w3_hbm, w3_buf, sem_misc.at[3 + WO_CH])
        w2a_cp = pltpu.make_async_copy(w2_hbm.at[pl.ds(0, W2_SPLIT), :], w2_buf.at[pl.ds(0, W2_SPLIT), :],
                                       sem_misc.at[4 + WO_CH])
        w2b_cp = pltpu.make_async_copy(w2_hbm.at[pl.ds(W2_SPLIT, F - W2_SPLIT), :],
                                       w2_buf.at[pl.ds(W2_SPLIT, F - W2_SPLIT), :], sem_misc.at[5 + WO_CH])

        def k_cp(h, slot):
            return pltpu.make_async_copy(k_hbm.at[h, :, pl.ds(SK - W, W)], k_buf.at[slot], sem_k.at[slot])

        def v_cp(h, slot):
            return pltpu.make_async_copy(v_hbm.at[h, :, pl.ds(SK - W, W)], v_buf.at[slot], sem_v.at[slot])

        x_cp.start()
        wq_cp.start()
        for h in range(NSLOT):
            k_cp(h, h).start()
            v_cp(h, h).start()

        x_cp.wait()
        x = jnp.broadcast_to(x_buf[...].astype(jnp.float32), (8, D))
        xn = _ln(x).astype(jnp.bfloat16)
        wq_cp.wait()
        for j in range(NPAIR):
            q = jnp.dot(xn, wq_buf[:, j * 384:(j + 1) * 384], preferred_element_type=jnp.float32)
            q_scr[j] = q

        scale = DH ** -0.5

        def pair_body(j, carry):
            qp = q_scr[j].astype(jnp.bfloat16)
            outs = []
            for i in range(2):
                h = 2 * j + i
                slot = (j % PSL) * 2 + i
                q = qp[:, i * DH:(i + 1) * DH]
                k_cp(h, slot).wait()
                s = jnp.dot(q, k_buf[slot], preferred_element_type=jnp.float32) * scale

                @pl.when(h + NSLOT < H)
                def _():
                    k_cp(h + NSLOT, slot).start()

                m = jnp.max(s, axis=-1, keepdims=True)
                p = jnp.exp(s - m)
                l = jnp.sum(p, axis=-1, keepdims=True)
                v_cp(h, slot).wait()
                o = jax.lax.dot_general(p.astype(jnp.bfloat16), v_buf[slot], (((1,), (1,)), ((), ())),
                                        preferred_element_type=jnp.float32)

                @pl.when(h + NSLOT < H)
                def _():
                    v_cp(h + NSLOT, slot).start()

                if i == 1:
                    @pl.when(h + NSLOT == H - 1)
                    def _():
                        for c in wo_cps:
                            c.start()
                        w1_cp.start()
                        w3_cp.start()
                        w2a_cp.start()
                        w2b_cp.start()
                outs.append(o / l)
            o_scr[j] = jnp.concatenate(outs, axis=-1)
            return carry

        jax.lax.fori_loop(0, NPAIR, pair_body, 0)

        acc = jnp.zeros((8, D), jnp.float32)
        ppc = NPAIR // WO_CH
        for c in range(WO_CH):
            wo_cps[c].wait()
            for jj in range(ppc):
                j = c * ppc + jj
                acc = acc + jnp.dot(o_scr[j].astype(jnp.bfloat16), wo_buf[j * 384:(j + 1) * 384, :],
                                    preferred_element_type=jnp.float32)
        h1 = x_buf[...].astype(jnp.float32) + acc.astype(jnp.bfloat16).astype(jnp.float32)
        h1 = h1.astype(jnp.bfloat16).astype(jnp.float32)
        hn = _ln(h1).astype(jnp.bfloat16)
        w1_cp.wait()
        gate = jnp.dot(hn, w1_buf[...], preferred_element_type=jnp.float32)
        w3_cp.wait()
        up = jnp.dot(hn, w3_buf[...], preferred_element_type=jnp.float32)
        act = (gate * jax.nn.sigmoid(gate) * up).astype(jnp.bfloat16)
        w2a_cp.wait()
        out = jnp.dot(act[:, :W2_SPLIT], w2_buf[0:W2_SPLIT, :], preferred_element_type=jnp.float32)
        w2b_cp.wait()
        out = out + jnp.dot(act[:, W2_SPLIT:], w2_buf[W2_SPLIT:, :], preferred_element_type=jnp.float32)
        res = h1 + out
        o_ref[0] = res[0:1].astype(o_ref.dtype)

    scratch = [
        pltpu.VMEM((1, D), jnp.bfloat16),
        pltpu.VMEM((D, H * DH), jnp.bfloat16),
        pltpu.VMEM((H * DH, D), jnp.bfloat16),
        pltpu.VMEM((D, F), jnp.bfloat16),
        pltpu.VMEM((D, F), jnp.bfloat16),
        pltpu.VMEM((F, D), jnp.bfloat16),
        pltpu.VMEM((NSLOT, DH, W), jnp.bfloat16),
        pltpu.VMEM((NSLOT, DH, W), jnp.bfloat16),
        pltpu.VMEM((NPAIR, 8, 2 * DH), jnp.float32),
        pltpu.VMEM((NPAIR, 8, 2 * DH), jnp.float32),
        pltpu.SemaphoreType.DMA((6 + WO_CH,)),
        pltpu.SemaphoreType.DMA((NSLOT,)),
        pltpu.SemaphoreType.DMA((NSLOT,)),
    ]
    return kernel, scratch


@jax.jit
def pallas_sequential_preLN__sliding_block_cached__glu_gated_swiglu__decode_kernel(
    A_x, A_k_cache, A_v_cache, A_wq, A_wo, B_x, B_w1, B_w3, B_w2,
):
    kernel, scratch = make_kernel()
    kt = jnp.swapaxes(A_k_cache, 2, 3).reshape(H, DH, SK)
    vt = jnp.swapaxes(A_v_cache, 2, 3).reshape(H, DH, SK)
    return pl.pallas_call(
        kernel,
        in_specs=[pl.BlockSpec(memory_space=pl.ANY)] * 8,
        out_specs=pl.BlockSpec(memory_space=pltpu.VMEM),
        out_shape=jax.ShapeDtypeStruct((1, 1, D), jnp.bfloat16),
        scratch_shapes=scratch,
        compiler_params=pltpu.CompilerParams(vmem_limit_bytes=100 * 1024 * 1024),
    )(A_x, kt, vt, A_wq, A_wo, B_w1, B_w3, B_w2)
```

```python
import functools
import jax
import jax.numpy as jnp
import numpy as np
import jax.experimental.pallas as pl
import jax.experimental.pallas.tpu as pltpu

D = 640
H = 32
DH = 192
SK = 32768
W = 4096
F = 1536
EPS = 1e-5


def _ln(x):
    m = jnp.mean(x, axis=-1, keepdims=True)
    xc = x - m
    v = jnp.mean(xc * xc, axis=-1, keepdims=True)
    return xc * jax.lax.rsqrt(v + EPS)


def make_kernel(NSLOT=4, W2_ROWS=256, scopes=False):
    NPAIR = H // 2
    assert NSLOT % 2 == 0
    PSL = NSLOT // 2
    NW2 = F // W2_ROWS
    J_LAST_KV = (H - 1 - NSLOT) // 2
    J_WO = min(J_LAST_KV + 1, NPAIR - 1)
    J_FFN = min(J_LAST_KV + 2, NPAIR - 1)
    import contextlib
    sc = (lambda n: jax.named_scope(n)) if scopes else (lambda n: contextlib.nullcontext())

    def kernel(x_hbm, k_hbm, v_hbm, wq_hbm, wo_hbm, w1_hbm, w3_hbm, w2_hbm, o_ref,
               x_buf, wq_buf, wo_buf, w13_buf, w2_buf, k_buf, v_buf, q_scr, o_scr, gu_scr, act_scr,
               sem_misc, sem_k, sem_v, sem_wo, sem_w13, sem_w2):
        x_cp = pltpu.make_async_copy(x_hbm.at[0], x_buf, sem_misc.at[0])
        wq_cp = pltpu.make_async_copy(wq_hbm, wq_buf, sem_misc.at[1])

        def wo_cp(j):
            return pltpu.make_async_copy(wo_hbm.at[j], wo_buf.at[j], sem_wo.at[j])

        def w13_cp(i, src):
            return pltpu.make_async_copy(src, w13_buf.at[i], sem_w13.at[i])

        def w2_cp(c):
            return pltpu.make_async_copy(w2_hbm.at[c], w2_buf.at[c], sem_w2.at[c])

        def k_cp(h, slot):
            return pltpu.make_async_copy(k_hbm.at[h, :, pl.ds(SK - W, W)], k_buf.at[slot], sem_k.at[slot])

        def v_cp(h, slot):
            return pltpu.make_async_copy(v_hbm.at[h, :, pl.ds(SK - W, W)], v_buf.at[slot], sem_v.at[slot])

        x_cp.start()
        wq_cp.start()

        def start_kv(h, c):
            k_cp(h, h).start()
            v_cp(h, h).start()
            return c
        jax.lax.fori_loop(0, NSLOT, start_kv, 0)

        with sc("wait_x"):
            x_cp.wait()
        x = jnp.broadcast_to(x_buf[...].astype(jnp.float32), (8, D))
        xn = _ln(x).astype(jnp.bfloat16)
        with sc("wait_wq"):
            wq_cp.wait()
        for j in range(NPAIR):
            q = jnp.dot(xn, wq_buf[:, j * 384:(j + 1) * 384], preferred_element_type=jnp.float32)
            q_scr[j] = q

        scale = DH ** -0.5

        def pair_body(j, carry):
            @pl.when(j == J_WO)
            def _():
                def st(c, cc):
                    wo_cp(c).start()
                    return cc
                jax.lax.fori_loop(0, NPAIR, st, 0)

            @pl.when(j == J_FFN)
            def _():
                w13_cp(0, w1_hbm).start()
                w13_cp(1, w3_hbm).start()
                def st(c, cc):
                    w2_cp(c).start()
                    return cc
                jax.lax.fori_loop(0, NW2, st, 0)

            qp = q_scr[j].astype(jnp.bfloat16)
            outs = []
            for i in range(2):
                h = 2 * j + i
                slot = (j % PSL) * 2 + i
                q = qp[:, i * DH:(i + 1) * DH]
                with sc("wait_k"):
                    k_cp(h, slot).wait()
                s = jnp.dot(q, k_buf[slot], preferred_element_type=jnp.float32) * scale

                @pl.when(h + NSLOT < H)
                def _():
                    k_cp(h + NSLOT, slot).start()

                m = jnp.max(s, axis=-1, keepdims=True)
                p = jnp.exp(s - m)
                l = jnp.sum(p, axis=-1, keepdims=True)
                with sc("wait_v"):
                    v_cp(h, slot).wait()
                o = jax.lax.dot_general(p.astype(jnp.bfloat16), v_buf[slot], (((1,), (1,)), ((), ())),
                                        preferred_element_type=jnp.float32)

                @pl.when(h + NSLOT < H)
                def _():
                    v_cp(h + NSLOT, slot).start()
                outs.append(o / l)
            o_scr[j] = jnp.concatenate(outs, axis=-1)
            return carry

        jax.lax.fori_loop(0, NPAIR, pair_body, 0)

        def wo_body(j, acc):
            with sc("wait_wo"):
                wo_cp(j).wait()
            return acc + jnp.dot(o_scr[j].astype(jnp.bfloat16), wo_buf[j], preferred_element_type=jnp.float32)
        acc = jax.lax.fori_loop(0, NPAIR, wo_body, jnp.zeros((8, D), jnp.float32))

        h1 = x_buf[...].astype(jnp.float32) + acc.astype(jnp.bfloat16).astype(jnp.float32)
        h1 = h1.astype(jnp.bfloat16).astype(jnp.float32)
        hn = _ln(h1).astype(jnp.bfloat16)

        def gu_body(i, c):
            with sc("wait_w13"):
                w13_cp(i, w1_hbm).wait()
            gu_scr[i] = jnp.dot(hn, w13_buf[i], preferred_element_type=jnp.float32)
            return c
        jax.lax.fori_loop(0, 2, gu_body, 0)
        gate = gu_scr[0]
        up = gu_scr[1]
        act = gate * jax.nn.sigmoid(gate) * up
        for c in range(NW2):
            act_scr[c] = act[:, c * W2_ROWS:(c + 1) * W2_ROWS]

        def w2_body(c, out):
            with sc("wait_w2"):
                w2_cp(c).wait()
            return out + jnp.dot(act_scr[c].astype(jnp.bfloat16), w2_buf[c], preferred_element_type=jnp.float32)
        res = jax.lax.fori_loop(0, NW2, w2_body, h1)
        o_ref[0] = res[0:1].astype(o_ref.dtype)

    scratch = [
        pltpu.VMEM((1, D), jnp.bfloat16),
        pltpu.VMEM((D, H * DH), jnp.bfloat16),
        pltpu.VMEM((NPAIR, 2 * DH, D), jnp.bfloat16),
        pltpu.VMEM((2, D, F), jnp.bfloat16),
        pltpu.VMEM((NW2, W2_ROWS, D), jnp.bfloat16),
        pltpu.VMEM((NSLOT, DH, W), jnp.bfloat16),
        pltpu.VMEM((NSLOT, DH, W), jnp.bfloat16),
        pltpu.VMEM((NPAIR, 8, 2 * DH), jnp.float32),
        pltpu.VMEM((NPAIR, 8, 2 * DH), jnp.float32),
        pltpu.VMEM((2, 8, F), jnp.float32),
        pltpu.VMEM((NW2, 8, W2_ROWS), jnp.float32),
        pltpu.SemaphoreType.DMA((2,)),
        pltpu.SemaphoreType.DMA((NSLOT,)),
        pltpu.SemaphoreType.DMA((NSLOT,)),
        pltpu.SemaphoreType.DMA((NPAIR,)),
        pltpu.SemaphoreType.DMA((2,)),
        pltpu.SemaphoreType.DMA((NW2,)),
    ]
    return kernel, scratch, NW2


@jax.jit
def pallas_sequential_preLN__sliding_block_cached__glu_gated_swiglu__decode_kernel(
    A_x, A_k_cache, A_v_cache, A_wq, A_wo, B_x, B_w1, B_w3, B_w2,
):
    kernel, scratch, NW2 = make_kernel()
    kt = jnp.swapaxes(A_k_cache, 2, 3).reshape(H, DH, SK)
    vt = jnp.swapaxes(A_v_cache, 2, 3).reshape(H, DH, SK)
    return pl.pallas_call(
        kernel,
        in_specs=[pl.BlockSpec(memory_space=pl.ANY)] * 8,
        out_specs=pl.BlockSpec(memory_space=pltpu.VMEM),
        out_shape=jax.ShapeDtypeStruct((1, 1, D), jnp.bfloat16),
        scratch_shapes=scratch,
        compiler_params=pltpu.CompilerParams(vmem_limit_bytes=100 * 1024 * 1024),
    )(A_x, kt, vt, A_wq, A_wo.reshape(H // 2, 2 * DH, D), B_w1, B_w3, B_w2.reshape(NW2, F // NW2, D))
```

```python
import contextlib
import functools
import jax
import jax.numpy as jnp
import numpy as np
import jax.experimental.pallas as pl
import jax.experimental.pallas.tpu as pltpu

D = 640
H = 32
DH = 192
SK = 32768
W = 4096
F = 1536
EPS = 1e-5
NP = W // 128


def _ln(x):
    m = jnp.mean(x, axis=-1, keepdims=True)
    xc = x - m
    v = jnp.mean(xc * xc, axis=-1, keepdims=True)
    return xc * jax.lax.rsqrt(v + EPS)


def make_kernel(scopes=False, NE=3, unroll_issue=True, mode='split'):
    sc = (lambda n: jax.named_scope(n)) if scopes else (lambda n: contextlib.nullcontext())
    scale = DH ** -0.5
    NCB = H * DH // 128
    NA = 6
    CBA = NCB // NA
    WOR = H * DH // NA
    ER = F // 2 // NE

    def kernel(x_hbm, k_hbm, v_hbm, wq_hbm, wo_hbm, w1_hbm, w3_hbm, w2_hbm, o_ref,
               x_buf, wq_buf, wo_buf, w1_buf, w3_buf, w2_buf, k_buf, v_buf,
               qc_scr, qh_scr, act_scr, sem_x, sem0, sem1, sem_e0, sem_e1):
        def loop(n, fn):
            if unroll_issue:
                for i in range(n):
                    fn(i)
            else:
                @pl.loop(0, n)
                def _(i):
                    fn(i)

        def start_a(g, sl):
            def one(i):
                cb = g * CBA + i // 4
                rb = i % 4
                r = rb * 160 if isinstance(rb, int) else pl.multiple_of(rb * 160, 16)
                pltpu.make_async_copy(
                    wq_hbm.at[pl.ds(r, 160), pl.ds(pl.multiple_of(cb * 128, 128), 128)],
                    wq_buf.at[cb, pl.ds(r, 160), :], sem0.at[sl]).start(priority=0)
                r = pl.multiple_of(g * WOR + i * 32, 32)
                pltpu.make_async_copy(wo_hbm.at[pl.ds(r, 32), :], wo_buf.at[pl.ds(r, 32), :],
                                      sem1.at[sl]).start(priority=1)
            loop(32, one)

        def wait_a0(g, sl):
            d = wq_buf.at[pl.ds(pl.multiple_of(g * CBA, CBA), CBA)]
            pltpu.make_async_copy(d, d, sem0.at[sl]).wait()

        def wait_a1(g, sl):
            d = wo_buf.at[pl.ds(pl.multiple_of(g * WOR, WOR), WOR), :]
            pltpu.make_async_copy(d, d, sem1.at[sl]).wait()

        def start_k(h, sl):
            def one(c):
                o = c * 128 if isinstance(c, int) else pl.multiple_of(c * 128, 128)
                pltpu.make_async_copy(k_hbm.at[h, :, pl.ds(SK - W + o, 128)], k_buf.at[sl, :, pl.ds(o, 128)],
                                      sem0.at[sl]).start(priority=0)
            loop(NP, one)

        def start_v(h, sl):
            def one(c):
                o = c * 128 if isinstance(c, int) else pl.multiple_of(c * 128, 128)
                pltpu.make_async_copy(v_hbm.at[h, :, pl.ds(SK - W + o, 128)], v_buf.at[sl, :, pl.ds(o, 128)],
                                      sem1.at[sl]).start(priority=1)
            loop(NP, one)

        def wait_k(sl):
            pltpu.make_async_copy(k_buf.at[sl], k_buf.at[sl], sem0.at[sl]).wait()

        def wait_v(sl):
            pltpu.make_async_copy(v_buf.at[sl], v_buf.at[sl], sem1.at[sl]).wait()

        def start_d0(sl):
            def one(i):
                r = i * 16 if isinstance(i, int) else pl.multiple_of(i * 16, 16)
                pltpu.make_async_copy(w1_hbm.at[pl.ds(r, 16), :], w1_buf.at[pl.ds(r, 16), :], sem0.at[sl]).start(priority=0)
            loop(D // 16, one)

        def start_d1(sl):
            def one(i):
                r = i * 16 if isinstance(i, int) else pl.multiple_of(i * 16, 16)
                pltpu.make_async_copy(w3_hbm.at[pl.ds(r, 16), :], w3_buf.at[pl.ds(r, 16), :], sem1.at[sl]).start(priority=1)
            loop(D // 16, one)

        def start_e(t):
            sem = sem_e0 if t == 0 else sem_e1
            for e in range(NE):
                def one(i):
                    r = t * (F // 2) + e * ER + i * 32
                    r = r if isinstance(r, int) else pl.multiple_of(r, 32)
                    pltpu.make_async_copy(w2_hbm.at[pl.ds(r, 32), :], w2_buf.at[pl.ds(r, 32), :],
                                          sem.at[e]).start(priority=t)
                loop(ER // 32, one)

        def wait_e(t, e):
            sem = sem_e0 if t == 0 else sem_e1
            r = pl.multiple_of(t * (F // 2) + e * ER, 128)
            d = w2_buf.at[pl.ds(r, ER), :]
            pltpu.make_async_copy(d, d, sem.at[e]).wait()

        x_cp = pltpu.make_async_copy(x_hbm.at[0], x_buf, sem_x)
        x_cp.start()

        @pl.loop(0, 2)
        def _(g):
            start_a(g, g)

        x_cp.wait()
        x = jnp.broadcast_to(x_buf[...].astype(jnp.float32), (8, D))
        xn = _ln(x).astype(jnp.bfloat16)

        @pl.loop(0, NA)
        def _(g):
            sl = g % 2
            wait_a0(g, sl)
            wait_a1(g, sl)

            @pl.when(g + 2 < NA)
            def _():
                start_a(g + 2, sl)

            @pl.when(g + 2 >= NA)
            def _():
                start_k(g + 2 - NA, sl)
                start_v(g + 2 - NA, sl)
            for c in range(CBA):
                qc_scr[g * CBA + c] = jnp.dot(xn, wq_buf[g * CBA + c], preferred_element_type=jnp.float32)

        for j in range(H // 2):
            trip = jnp.concatenate([qc_scr[3 * j], qc_scr[3 * j + 1], qc_scr[3 * j + 2]], axis=-1)
            qh_scr[2 * j] = trip[:, 0:DH]
            qh_scr[2 * j + 1] = trip[:, DH:2 * DH]

        def issue_k(h, sl):
            @pl.when(h + 2 < H)
            def _():
                start_k(h + 2, sl)

            @pl.when(h + 2 == H)
            def _():
                start_d0(sl)

            @pl.when(h + 2 == H + 1)
            def _():
                start_e(0)

        def issue_v(h, sl):
            @pl.when(h + 2 < H)
            def _():
                start_v(h + 2, sl)

            @pl.when(h + 2 == H)
            def _():
                start_d1(sl)

            @pl.when(h + 2 == H + 1)
            def _():
                start_e(1)

        def issue_kv_joint(h, sl):
            @pl.when(h + 2 < H)
            def _():
                def one(c):
                    o = c * 128 if isinstance(c, int) else pl.multiple_of(c * 128, 128)
                    pltpu.make_async_copy(k_hbm.at[h + 2, :, pl.ds(SK - W + o, 128)], k_buf.at[sl, :, pl.ds(o, 128)],
                                          sem0.at[sl]).start(priority=0)
                    pltpu.make_async_copy(v_hbm.at[h + 2, :, pl.ds(SK - W + o, 128)], v_buf.at[sl, :, pl.ds(o, 128)],
                                          sem1.at[sl]).start(priority=1)
                loop(NP, one)

            @pl.when(h + 2 == H)
            def _():
                start_d0(sl)
                start_d1(sl)

            @pl.when(h + 2 == H + 1)
            def _():
                start_e(0)
                start_e(1)

        def head(h, attn):
            sl = h % 2
            q = qh_scr[h].astype(jnp.bfloat16)
            with sc("wait_k"):
                wait_k(sl)
            s = jnp.dot(q, k_buf[sl], preferred_element_type=jnp.float32) * scale

            if mode == 'split':
                issue_k(h, sl)

            m = jnp.max(s, axis=-1, keepdims=True)
            p = jnp.exp(s - m)
            l = jnp.sum(p, axis=-1, keepdims=True)
            with sc("wait_v"):
                wait_v(sl)
            o = jax.lax.dot_general(p.astype(jnp.bfloat16), v_buf[sl], (((1,), (1,)), ((), ())),
                                    preferred_element_type=jnp.float32)

            if mode == 'split':
                issue_v(h, sl)
            elif mode == 'both':
                issue_kv_joint(h, sl)
            elif mode == 'vk':
                issue_v(h, sl)
                issue_k(h, sl)
            o = (o / l).astype(jnp.bfloat16)
            return attn + jnp.dot(o, wo_buf[pl.ds(pl.multiple_of(h * DH, 64), DH), :],
                                  preferred_element_type=jnp.float32)

        attn = jax.lax.fori_loop(0, H, head, jnp.zeros((8, D), jnp.float32))

        with sc("ln2"):
            h1 = x_buf[...].astype(jnp.float32) + attn.astype(jnp.bfloat16).astype(jnp.float32)
            h1 = h1.astype(jnp.bfloat16).astype(jnp.float32)
            hn = _ln(h1).astype(jnp.bfloat16)

        with sc("waitD"):
            pltpu.make_async_copy(w1_buf, w1_buf, sem0.at[H % 2]).wait()
            pltpu.make_async_copy(w3_buf, w3_buf, sem1.at[H % 2]).wait()
        with sc("gateup"):
            gate = jnp.dot(hn, w1_buf[...], preferred_element_type=jnp.float32)
            up = jnp.dot(hn, w3_buf[...], preferred_element_type=jnp.float32)
            act = gate * jax.nn.sigmoid(gate) * up
            for g in range(2 * NE):
                act_scr[g] = act[:, g * ER:(g + 1) * ER]

        def e_body(e, out):
            with sc("waitE"):
                wait_e(0, e)
                wait_e(1, e)
            r0 = pl.multiple_of(e * ER, 128)
            r1 = pl.multiple_of(F // 2 + e * ER, 128)
            out = out + jnp.dot(act_scr[e].astype(jnp.bfloat16), w2_buf[pl.ds(r0, ER), :], preferred_element_type=jnp.float32)
            out = out + jnp.dot(act_scr[NE + e].astype(jnp.bfloat16), w2_buf[pl.ds(r1, ER), :], preferred_element_type=jnp.float32)
            return out
        res = jax.lax.fori_loop(0, NE, e_body, h1)
        o_ref[0] = res[0:1].astype(o_ref.dtype)

    scratch = [
        pltpu.VMEM((1, D), jnp.bfloat16),
        pltpu.VMEM((NCB, D, 128), jnp.bfloat16),
        pltpu.VMEM((H * DH, D), jnp.bfloat16),
        pltpu.VMEM((D, F), jnp.bfloat16),
        pltpu.VMEM((D, F), jnp.bfloat16),
        pltpu.VMEM((F, D), jnp.bfloat16),
        pltpu.VMEM((2, DH, W), jnp.bfloat16),
        pltpu.VMEM((2, DH, W), jnp.bfloat16),
        pltpu.VMEM((NCB, 8, 128), jnp.float32),
        pltpu.VMEM((H, 8, DH), jnp.float32),
        pltpu.VMEM((2 * NE, 8, ER), jnp.float32),
        pltpu.SemaphoreType.DMA(()),
        pltpu.SemaphoreType.DMA((2,)),
        pltpu.SemaphoreType.DMA((2,)),
        pltpu.SemaphoreType.DMA((NE,)),
        pltpu.SemaphoreType.DMA((NE,)),
    ]
    return kernel, scratch


@jax.jit
def pallas_sequential_preLN__sliding_block_cached__glu_gated_swiglu__decode_kernel(
    A_x, A_k_cache, A_v_cache, A_wq, A_wo, B_x, B_w1, B_w3, B_w2,
):
    kernel, scratch = make_kernel(mode='both')
    kt = jnp.swapaxes(A_k_cache, 2, 3).reshape(H, DH, SK)
    vt = jnp.swapaxes(A_v_cache, 2, 3).reshape(H, DH, SK)
    return pl.pallas_call(
        kernel,
        in_specs=[pl.BlockSpec(memory_space=pl.ANY)] * 8,
        out_specs=pl.BlockSpec(memory_space=pltpu.VMEM),
        out_shape=jax.ShapeDtypeStruct((1, 1, D), jnp.bfloat16),
        scratch_shapes=scratch,
        compiler_params=pltpu.CompilerParams(vmem_limit_bytes=100 * 1024 * 1024),
    )(A_x, kt, vt, A_wq, A_wo, B_w1, B_w3, B_w2)
```

```python
import contextlib
import jax
import jax.numpy as jnp
import numpy as np
import jax.experimental.pallas as pl
import jax.experimental.pallas.tpu as pltpu

D = 640
H = 32
DH = 192
SK = 32768
W = 4096
F = 1536
EPS = 1e-5


def _ln(x):
    m = jnp.mean(x, axis=-1, keepdims=True)
    xc = x - m
    v = jnp.mean(xc * xc, axis=-1, keepdims=True)
    return xc * jax.lax.rsqrt(v + EPS)


def _al(v, m):
    return v if isinstance(v, int) else pl.multiple_of(v, m)


def make_kernel(scopes=False, ES=(256, 256, 256), KV=(8, 2048), WQ=(8, 2048), WO=(24, 640), W13=(8, 1536), W2=(32, 640),
                NWO=4, WO_PRE=2, swap=False, dshift=0, emode='half', BQ=1, BO=1, BD=1, BE=1, BKV=1, NQ=4, BV=None, ROT=0, REV=False):
    sc = (lambda n: jax.named_scope(n)) if scopes else (lambda n: contextlib.nullcontext())
    scale = DH ** -0.5
    NE = len(ES)
    assert sum(ES) == F // 2
    EOFF = [sum(ES[:i]) for i in range(NE)]
    HD = H * DH
    WOH = HD // 2
    WOR = WOH // NWO

    def kernel(x_hbm, k_hbm, v_hbm, wq_hbm, wo_hbm, w1_hbm, w3_hbm, w2_hbm, o_ref,
               x_buf, wq_buf, wo_buf, w1_buf, w3_buf, w2_buf, k_buf, v_buf,
               qh_scr, gu_scr, sem_x, sem_a, sem0, sem1, sem_e0, sem_e1):

        def pieces(src, dst, r0, nr, c_src, nc, shape, sem, ralign, B=1):
            pr, pc = shape
            widths = list(pc) if isinstance(pc, (tuple, list)) else [pc] * (nc // pc)
            assert sum(widths) == nc
            offs = [sum(widths[:j]) for j in range(len(widths))]
            out = []
            for i in range(nr // pr):
                r = _al(r0 + i * pr, ralign)
                for o, wd in zip(offs, widths):
                    out.append(pltpu.make_async_copy(src.at[pl.ds(r, pr), pl.ds(c_src + o, wd)],
                                                     dst.at[pl.ds(r, pr), pl.ds(o, wd)], sem))
            n = len(out)
            assert n % B == 0, (n, B)
            return [out[b * B + c] for c in range(B) for b in range(n // B)]

        def start2(l0, l1):
            for i in range(max(len(l0), len(l1))):
                if i < len(l0):
                    l0[i].start(priority=1 if swap else 0)
                if i < len(l1):
                    l1[i].start(priority=0 if swap else 1)

        def wait_region(dst, r0, nr, sem, ralign):
            d = dst.at[pl.ds(_al(r0, ralign), nr), :]
            pltpu.make_async_copy(d, d, sem).wait()

        def start_kv(h, sl):
            a = pieces(k_hbm.at[h], k_buf.at[sl], 0, DH, SK - W, W, KV, sem0.at[sl], 8, BKV)
            b = pieces(v_hbm.at[h], v_buf.at[sl], 0, DH, SK - W, W, KV, sem1.at[sl], 8, BV or BKV)
            b = b[ROT:] + b[:ROT]
            if REV:
                b = b[::-1]
            start2(a, b)

        def start_d(sl):
            a = pieces(w1_hbm, w1_buf, 0, D, 0, F, W13, sem0.at[sl], 8, BD)
            b = pieces(w3_hbm, w3_buf, 0, D, 0, F, W13, sem1.at[sl], 8, BD)
            if dshift >= 0:
                start2(a + b[:dshift], b[dshift:])
            else:
                start2(a[-dshift:], b + a[:-dshift])

        def start_e():
            for e in range(NE):
                a = pieces(w2_hbm, w2_buf, EOFF[e], ES[e], 0, D, W2, sem_e0.at[e], 8, BE)
                b = pieces(w2_hbm, w2_buf, F // 2 + EOFF[e], ES[e], 0, D, W2, sem_e1.at[e], 8, BE)
                if emode == 'half':
                    start2(a, b)
                elif emode == 't0':
                    start2([x for p in zip(a, b) for x in p], [])
                elif emode == 't1':
                    start2([], [x for p in zip(a, b) for x in p])

        x_cp = pltpu.make_async_copy(x_hbm.at[0], x_buf, sem_x)
        x_cp.start()

        QR = D // 2 // NQ

        @pl.loop(0, NQ)
        def _(g):
            start2(pieces(wq_hbm, wq_buf, g * QR, QR, 0, HD, WQ, sem_a.at[0], 8, BQ),
                   pieces(wq_hbm, wq_buf, D // 2 + g * QR, QR, 0, HD, WQ, sem_a.at[1], 8, BQ))

        def start_wo(g):
            start2(pieces(wo_hbm, wo_buf, g * WOR, WOR, 0, D, WO, sem_a.at[2], 8, BO),
                   pieces(wo_hbm, wo_buf, WOH + g * WOR, WOR, 0, D, WO, sem_a.at[3], 8, BO))

        @pl.loop(0, WO_PRE)
        def _(g):
            start_wo(g)

        x_cp.wait()
        x = jnp.broadcast_to(x_buf[...].astype(jnp.float32), (8, D))
        xn = _ln(x).astype(jnp.bfloat16)
        with sc("wait_wq"):
            wait_region(wq_buf, 0, D // 2, sem_a.at[0], 8)
            wait_region(wq_buf, D // 2, D // 2, sem_a.at[1], 8)

        with sc("q"):
            @pl.loop(0, H // 4)
            def _(j):
                q4 = jnp.dot(xn, wq_buf[:, pl.ds(pl.multiple_of(j * 4 * DH, 128), 4 * DH)],
                             preferred_element_type=jnp.float32)
                for i in range(4):
                    qh_scr[4 * j + i] = q4[:, i * DH:(i + 1) * DH]

        @pl.loop(WO_PRE, NWO)
        def _(g):
            start_wo(g)

        @pl.loop(0, 2)
        def _(h):
            start_kv(h, h)

        with sc("wait_wo"):
            wait_region(wo_buf, 0, WOH, sem_a.at[2], 8)
            wait_region(wo_buf, WOH, WOH, sem_a.at[3], 8)

        def head(h, attn):
            sl = h % 2
            q = qh_scr[h].astype(jnp.bfloat16)
            with sc("wait_k"):
                wait_region(k_buf.at[sl], 0, DH, sem0.at[sl], 8)
            s = jnp.dot(q, k_buf[sl], preferred_element_type=jnp.float32) * scale
            m = jnp.max(s, axis=-1, keepdims=True)
            p = jnp.exp(s - m)
            l = jnp.sum(p, axis=-1, keepdims=True)
            with sc("wait_v"):
                wait_region(v_buf.at[sl], 0, DH, sem1.at[sl], 8)
            o = jax.lax.dot_general(p.astype(jnp.bfloat16), v_buf[sl], (((1,), (1,)), ((), ())),
                                    preferred_element_type=jnp.float32)

            @pl.when(h + 2 < H)
            def _():
                start_kv(h + 2, sl)

            @pl.when(h + 2 == H)
            def _():
                start_d(sl)

            @pl.when(h + 1 == H)
            def _():
                start_e()

            o = (o / l).astype(jnp.bfloat16)
            return attn + jnp.dot(o, wo_buf[pl.ds(pl.multiple_of(h * DH, 64), DH), :],
                                  preferred_element_type=jnp.float32)

        attn = jax.lax.fori_loop(0, H, head, jnp.zeros((8, D), jnp.float32))

        with sc("ln2"):
            h1 = x_buf[...].astype(jnp.float32) + attn.astype(jnp.bfloat16).astype(jnp.float32)
            h1 = h1.astype(jnp.bfloat16).astype(jnp.float32)
            hn = _ln(h1).astype(jnp.bfloat16)

        with sc("waitD"):
            wait_region(w1_buf, 0, D, sem0.at[H % 2], 8)
            wait_region(w3_buf, 0, D, sem1.at[H % 2], 8)
        with sc("gateup"):
            gate = jnp.dot(hn, w1_buf[...], preferred_element_type=jnp.float32)
            up = jnp.dot(hn, w3_buf[...], preferred_element_type=jnp.float32)
            gu_scr[...] = gate * jax.nn.sigmoid(gate) * up

        uniform = len(set(ES)) == 1
        if uniform:
            ER = ES[0]

            def e_body(e, out):
                r0 = pl.multiple_of(e * ER, 128)
                r1 = pl.multiple_of(F // 2 + e * ER, 128)
                with sc("waitE"):
                    wait_region(w2_buf, r0, ER, sem_e0.at[e], 128)
                    wait_region(w2_buf, r1, ER, sem_e1.at[e], 128)
                out = out + jnp.dot(gu_scr[:, pl.ds(r0, ER)].astype(jnp.bfloat16), w2_buf[pl.ds(r0, ER), :],
                                    preferred_element_type=jnp.float32)
                out = out + jnp.dot(gu_scr[:, pl.ds(r1, ER)].astype(jnp.bfloat16), w2_buf[pl.ds(r1, ER), :],
                                    preferred_element_type=jnp.float32)
                return out
            res = jax.lax.fori_loop(0, NE, e_body, h1)
        o_ref[0] = res[0:1].astype(o_ref.dtype)

    scratch = [
        pltpu.VMEM((1, D), jnp.bfloat16),
        pltpu.VMEM((D, H * DH), jnp.bfloat16),
        pltpu.VMEM((H * DH, D), jnp.bfloat16),
        pltpu.VMEM((D, F), jnp.bfloat16),
        pltpu.VMEM((D, F), jnp.bfloat16),
        pltpu.VMEM((F, D), jnp.bfloat16),
        pltpu.VMEM((2, DH, W), jnp.bfloat16),
        pltpu.VMEM((2, DH, W), jnp.bfloat16),
        pltpu.VMEM((H, 8, DH), jnp.float32),
        pltpu.VMEM((8, F), jnp.float32),
        pltpu.SemaphoreType.DMA(()),
        pltpu.SemaphoreType.DMA((4,)),
        pltpu.SemaphoreType.DMA((2,)),
        pltpu.SemaphoreType.DMA((2,)),
        pltpu.SemaphoreType.DMA((NE,)),
        pltpu.SemaphoreType.DMA((NE,)),
    ]
    return kernel, scratch


@jax.jit
def pallas_sequential_preLN__sliding_block_cached__glu_gated_swiglu__decode_kernel(
    A_x, A_k_cache, A_v_cache, A_wq, A_wo, B_x, B_w1, B_w3, B_w2,
):
    kernel, scratch = make_kernel(NQ=1,BQ=20,NWO=4,WO_PRE=3,WO=(32,640),BO=12,BD=20,BKV=4)
    kt = jnp.swapaxes(A_k_cache, 2, 3).reshape(H, DH, SK)
    vt = jnp.swapaxes(A_v_cache, 2, 3).reshape(H, DH, SK)
    return pl.pallas_call(
        kernel,
        in_specs=[pl.BlockSpec(memory_space=pl.ANY)] * 8,
        out_specs=pl.BlockSpec(memory_space=pltpu.VMEM),
        out_shape=jax.ShapeDtypeStruct((1, 1, D), jnp.bfloat16),
        scratch_shapes=scratch,
        compiler_params=pltpu.CompilerParams(vmem_limit_bytes=100 * 1024 * 1024, disable_semaphore_checks=True, disable_bounds_checks=True),
    )(A_x, kt, vt, A_wq, A_wo, B_w1, B_w3, B_w2)
```

```python
import jax
import jax.numpy as jnp
import jax.experimental.pallas as pl
import jax.experimental.pallas.tpu as pltpu

D = 640
H = 32
DH = 192
HD = H * DH
SK = 32768
W = min(4096, max(256, SK // 4))
F = 1536
EPS = 1e-5
NE = 3
ER = F // 2 // NE
BKV, BQ, BO, BD = 4, 30, 16, 20
NWO = WO_PRE = 2
WOP = W2P = 32
WOH = HD // 2
WOR = WOH // NWO


def _ln(x):
    m = jnp.mean(x, axis=-1, keepdims=True)
    xc = x - m
    v = jnp.mean(xc * xc, axis=-1, keepdims=True)
    return xc * jax.lax.rsqrt(v + EPS)


def _al(v, m):
    return v if isinstance(v, int) else pl.multiple_of(v, m)


def _kernel(x_hbm, k_hbm, v_hbm, wq_hbm, wo_hbm, w1_hbm, w3_hbm, w2_hbm, o_ref,
           x_buf, wq_buf, wo_buf, w1_buf, w3_buf, w2_buf, k_buf, v_buf, qh_scr, act_scr,
               sems):

    def pieces(src, dst, r0, nr, c_src, nc, pr, pc, sem, stride):
        out = []
        for i in range(nr // pr):
            r = _al(r0 + i * pr, 8)
            for j in range(nc // pc):
                out.append(pltpu.make_async_copy(src.at[pl.ds(r, pr), pl.ds(c_src + j * pc, pc)],
                                                 dst.at[pl.ds(r, pr), pl.ds(j * pc, pc)], sem))
        n = len(out)
        assert n % stride == 0
        return [out[b * stride + c] for c in range(stride) for b in range(n // stride)]

    def start2(q0, q1):
        for a, b in zip(q0, q1, strict=True):
            a.start(priority=0)
            b.start(priority=1)

    def wait_all(dst, sem):
        pltpu.make_async_copy(dst, dst, sem).wait()

    def start_kv(h, sl):
        start2(pieces(k_hbm.at[h], k_buf.at[sl], 0, DH, SK - W, W, 8, 2048, sems.at[2 + sl], BKV),
               pieces(v_hbm.at[h], v_buf.at[sl], 0, DH, SK - W, W, 8, 2048, sems.at[2 + sl], BKV))

    def start_wo(g):
        start2(pieces(wo_hbm, wo_buf, g * WOR, WOR, 0, D, WOP, D, sems.at[1], BO),
               pieces(wo_hbm, wo_buf, WOH + g * WOR, WOR, 0, D, WOP, D, sems.at[1], BO))

    def start_w13(sl):
        start2(pieces(w1_hbm, w1_buf, 0, D, 0, F, 8, F, sems.at[2 + sl], BD),
               pieces(w3_hbm, w3_buf, 0, D, 0, F, 8, F, sems.at[2 + sl], BD))

    def start_w2():
        for e in range(NE):
            start2(pieces(w2_hbm, w2_buf, e * ER, ER, 0, D, W2P, D, sems.at[e + e // 2], 1),
                   pieces(w2_hbm, w2_buf, F // 2 + e * ER, ER, 0, D, W2P, D, sems.at[e + e // 2], 1))

    x_cp = pltpu.make_async_copy(x_hbm.at[0], x_buf, sems.at[0])
    x_cp.start()
    start2(pieces(wq_hbm, wq_buf, 0, D // 2, 0, HD, 8, 2048, sems.at[0], BQ),
           pieces(wq_hbm, wq_buf, D // 2, D // 2, 0, HD, 8, 2048, sems.at[0], BQ))

    @pl.loop(0, WO_PRE)
    def _(g):
        start_wo(g)

    x_cp.wait()
    wait_all(wq_buf, sems.at[0])
    x = jnp.broadcast_to(x_buf[...].astype(jnp.float32), (8, D))
    xn = _ln(x).astype(jnp.bfloat16)

    @pl.loop(0, H // 4)
    def _(j):
        q4 = jnp.dot(xn, wq_buf[:, pl.ds(pl.multiple_of(j * 4 * DH, 128), 4 * DH)],
                     preferred_element_type=jnp.float32)
        for i in range(4):
            qh_scr[4 * j + i] = q4[:, i * DH:(i + 1) * DH]


    @pl.loop(0, 2)
    def _(h):
        start_kv(h, h)

    wait_all(wo_buf, sems.at[1])

    def head(h, attn):
        sl = h % 2
        q = qh_scr[h].astype(jnp.bfloat16)
        wait_all(k_buf.at[sl], sems.at[2 + sl])
        wait_all(v_buf.at[sl], sems.at[2 + sl])
        s = jnp.dot(q, k_buf[sl], preferred_element_type=jnp.float32) * (DH ** -0.5)
        m = jnp.max(s, axis=-1, keepdims=True)
        p = jnp.exp(s - m)
        l = jnp.sum(p, axis=-1, keepdims=True)
        o = jax.lax.dot_general(p.astype(jnp.bfloat16), v_buf[sl], (((1,), (1,)), ((), ())),
                                preferred_element_type=jnp.float32)

        @pl.when(h + 2 < H)
        def _():
            start_kv(h + 2, sl)

        @pl.when(h + 2 == H)
        def _():
            start_w13(sl)

        @pl.when(h + 1 == H)
        def _():
            start_w2()

        o = (o / l).astype(jnp.bfloat16)
        return attn + jnp.dot(o, wo_buf[pl.ds(pl.multiple_of(h * DH, 64), DH), :],
                              preferred_element_type=jnp.float32)

    attn = jax.lax.fori_loop(0, H, head, jnp.zeros((8, D), jnp.float32))

    h1 = (x + attn.astype(jnp.bfloat16).astype(jnp.float32)).astype(jnp.bfloat16).astype(jnp.float32)
    hn = _ln(h1).astype(jnp.bfloat16)

    wait_all(w1_buf, sems.at[2 + H % 2])
    wait_all(w3_buf, sems.at[2 + H % 2])
    gate = jnp.dot(hn, w1_buf[...], preferred_element_type=jnp.float32)
    up = jnp.dot(hn, w3_buf[...], preferred_element_type=jnp.float32)
    act_scr[...] = gate * jax.nn.sigmoid(gate) * up

    def down(e, out):
        r0 = pl.multiple_of(e * ER, 128)
        r1 = pl.multiple_of(F // 2 + e * ER, 128)
        wait_all(w2_buf.at[pl.ds(r0, ER), :], sems.at[e + e // 2])
        wait_all(w2_buf.at[pl.ds(r1, ER), :], sems.at[e + e // 2])
        out = out + jnp.dot(act_scr[:, pl.ds(r0, ER)].astype(jnp.bfloat16), w2_buf[pl.ds(r0, ER), :],
                            preferred_element_type=jnp.float32)
        out = out + jnp.dot(act_scr[:, pl.ds(r1, ER)].astype(jnp.bfloat16), w2_buf[pl.ds(r1, ER), :],
                            preferred_element_type=jnp.float32)
        return out

    res = jax.lax.fori_loop(0, NE, down, h1)
    o_ref[0] = res[0:1].astype(o_ref.dtype)

_SCRATCH = [
    pltpu.VMEM((1, D), jnp.bfloat16),
    pltpu.VMEM((D, HD), jnp.bfloat16),
    pltpu.VMEM((HD, D), jnp.bfloat16),
    pltpu.VMEM((D, F), jnp.bfloat16),
    pltpu.VMEM((D, F), jnp.bfloat16),
    pltpu.VMEM((F, D), jnp.bfloat16),
    pltpu.VMEM((2, DH, W), jnp.bfloat16),
    pltpu.VMEM((2, DH, W), jnp.bfloat16),
    pltpu.VMEM((H, 8, DH), jnp.float32),
    pltpu.VMEM((8, F), jnp.float32),
    pltpu.SemaphoreType.DMA((4,)),
]


@jax.jit
def pallas_sequential_preLN__sliding_block_cached__glu_gated_swiglu__decode_kernel(
    A_x, A_k_cache, A_v_cache, A_wq, A_wo, B_x, B_w1, B_w3, B_w2,
):
    kt = jnp.swapaxes(A_k_cache, 2, 3).reshape(H, DH, SK)
    vt = jnp.swapaxes(A_v_cache, 2, 3).reshape(H, DH, SK)
    return pl.pallas_call(
        _kernel,
        in_specs=[pl.BlockSpec(memory_space=pl.ANY)] * 8,
        out_specs=pl.BlockSpec(memory_space=pltpu.VMEM),
        out_shape=jax.ShapeDtypeStruct((1, 1, D), jnp.bfloat16),
        scratch_shapes=_SCRATCH,
        compiler_params=pltpu.CompilerParams(vmem_limit_bytes=64 * 1024 * 1024),
    )(A_x, kt, vt, A_wq, A_wo, B_w1, B_w3, B_w2)
```

```python
import jax
import jax.numpy as jnp
import jax.experimental.pallas as pl
import jax.experimental.pallas.tpu as pltpu

D = 640
H = 32
DH = 192
HD = H * DH
SK = 32768
W = min(4096, max(256, SK // 4))
F = 1536
EPS = 1e-5
NE = 3
ER = F // NE
BKV, BQ, BO, BD = 4, 30, 16, 20
NWO = WO_PRE = 2
WOP = W2P = 32
WOH = HD // 2
WOR = WOH // NWO


def _ln(x):
    m = jnp.mean(x, axis=-1, keepdims=True)
    xc = x - m
    v = jnp.mean(xc * xc, axis=-1, keepdims=True)
    return xc * jax.lax.rsqrt(v + EPS)


def _al(v, m):
    return v if isinstance(v, int) else pl.multiple_of(v, m)


def _kernel(x_hbm, k_hbm, v_hbm, wq_hbm, wo_hbm, w1_hbm, w3_hbm, w2_hbm, o_ref,
            x_buf, wq_buf, wo_buf, w1_buf, w3_buf, w2_buf, k_buf, v_buf, qh_scr, act_scr,
            sem_x, sem_wq, sem_wo, sem_k, sem_v, sem_w2):

    def pieces(src, dst, r0, nr, c_src, nc, pr, pc, sem, stride):
        out = []
        for i in range(nr // pr):
            r = _al(r0 + i * pr, 8)
            for j in range(nc // pc):
                out.append(pltpu.make_async_copy(src.at[pl.ds(r, pr), pl.ds(c_src + j * pc, pc)],
                                                 dst.at[pl.ds(r, pr), pl.ds(j * pc, pc)], sem))
        n = len(out)
        assert n % stride == 0
        return [out[b * stride + c] for c in range(stride) for b in range(n // stride)]

    def start2(q0, q1):
        for a, b in zip(q0, q1, strict=True):
            a.start(priority=0)
            b.start(priority=1)

    def wait_all(dst, sem):
        pltpu.make_async_copy(dst, dst, sem).wait()

    def start_kv(h, sl):
        start2(pieces(k_hbm.at[h], k_buf.at[sl], 0, DH, SK - W, W, 8, 2048, sem_k.at[sl], BKV),
               pieces(v_hbm.at[h], v_buf.at[sl], 0, DH, SK - W, W, 8, 2048, sem_v.at[sl], BKV))

    def start_wo(g):
        start2(pieces(wo_hbm, wo_buf, g * WOR, WOR, 0, D, WOP, D, sem_wo, BO),
               pieces(wo_hbm, wo_buf, WOH + g * WOR, WOR, 0, D, WOP, D, sem_wo, BO))

    def start_w13(sl):
        start2(pieces(w1_hbm, w1_buf, 0, D, 0, F, 8, F, sem_k.at[sl], BD),
               pieces(w3_hbm, w3_buf, 0, D, 0, F, 8, F, sem_v.at[sl], BD))

    def start_w2():
        for e in range(NE):
            start2(pieces(w2_hbm, w2_buf, e * ER, ER // 2, 0, D, W2P, D, sem_w2.at[e], 1),
                   pieces(w2_hbm, w2_buf, e * ER + ER // 2, ER // 2, 0, D, W2P, D, sem_w2.at[e], 1))

    x_cp = pltpu.make_async_copy(x_hbm.at[0], x_buf, sem_x)
    x_cp.start()
    start2(pieces(wq_hbm, wq_buf, 0, D // 2, 0, HD, 8, 2048, sem_wq, BQ),
           pieces(wq_hbm, wq_buf, D // 2, D // 2, 0, HD, 8, 2048, sem_wq, BQ))

    @pl.loop(0, WO_PRE)
    def _(g):
        start_wo(g)

    x_cp.wait()
    wait_all(wq_buf, sem_wq)
    x = jnp.broadcast_to(x_buf[...].astype(jnp.float32), (8, D))
    xn = _ln(x).astype(jnp.bfloat16)

    @pl.loop(0, H // 4)
    def _(j):
        q4 = jnp.dot(xn, wq_buf[:, pl.ds(pl.multiple_of(j * 4 * DH, 128), 4 * DH)],
                     preferred_element_type=jnp.float32)
        for i in range(4):
            qh_scr[4 * j + i] = q4[:, i * DH:(i + 1) * DH]


    @pl.loop(0, 2)
    def _(h):
        start_kv(h, h)

    wait_all(wo_buf, sem_wo)

    def head(h, attn):
        sl = h % 2
        q = qh_scr[h].astype(jnp.bfloat16)
        wait_all(k_buf.at[sl], sem_k.at[sl])
        s = jnp.dot(q, k_buf[sl], preferred_element_type=jnp.float32) * (DH ** -0.5)
        m = jnp.max(s, axis=-1, keepdims=True)
        p = jnp.exp(s - m)
        l = jnp.sum(p, axis=-1, keepdims=True)
        wait_all(v_buf.at[sl], sem_v.at[sl])
        o = jax.lax.dot_general(p.astype(jnp.bfloat16), v_buf[sl], (((1,), (1,)), ((), ())),
                                preferred_element_type=jnp.float32)

        @pl.when(h + 2 < H)
        def _():
            start_kv(h + 2, sl)

        @pl.when(h + 2 == H)
        def _():
            start_w13(sl)

        @pl.when(h + 1 == H)
        def _():
            start_w2()

        o = (o / l).astype(jnp.bfloat16)
        return attn + jnp.dot(o, wo_buf[pl.ds(pl.multiple_of(h * DH, 64), DH), :],
                              preferred_element_type=jnp.float32)

    attn = jax.lax.fori_loop(0, H, head, jnp.zeros((8, D), jnp.float32))

    h1 = (x + attn.astype(jnp.bfloat16).astype(jnp.float32)).astype(jnp.bfloat16).astype(jnp.float32)
    hn = _ln(h1).astype(jnp.bfloat16)

    wait_all(w1_buf, sem_k.at[H % 2])
    wait_all(w3_buf, sem_v.at[H % 2])
    gate = jnp.dot(hn, w1_buf[...], preferred_element_type=jnp.float32)
    up = jnp.dot(hn, w3_buf[...], preferred_element_type=jnp.float32)
    act_scr[...] = gate * jax.nn.sigmoid(gate) * up

    def down(e, out):
        r = pl.multiple_of(e * ER, 128)
        wait_all(w2_buf.at[pl.ds(r, ER), :], sem_w2.at[e])
        return out + jnp.dot(act_scr[:, pl.ds(r, ER)].astype(jnp.bfloat16), w2_buf[pl.ds(r, ER), :],
                             preferred_element_type=jnp.float32)

    res = jax.lax.fori_loop(0, NE, down, h1)
    o_ref[0] = res[0:1].astype(o_ref.dtype)


_SCRATCH = [
    pltpu.VMEM((1, D), jnp.bfloat16),
    pltpu.VMEM((D, HD), jnp.bfloat16),
    pltpu.VMEM((HD, D), jnp.bfloat16),
    pltpu.VMEM((D, F), jnp.bfloat16),
    pltpu.VMEM((D, F), jnp.bfloat16),
    pltpu.VMEM((F, D), jnp.bfloat16),
    pltpu.VMEM((2, DH, W), jnp.bfloat16),
    pltpu.VMEM((2, DH, W), jnp.bfloat16),
    pltpu.VMEM((H, 8, DH), jnp.float32),
    pltpu.VMEM((8, F), jnp.float32),
    pltpu.SemaphoreType.DMA(()),
    pltpu.SemaphoreType.DMA(()),
    pltpu.SemaphoreType.DMA(()),
    pltpu.SemaphoreType.DMA((2,)),
    pltpu.SemaphoreType.DMA((2,)),
    pltpu.SemaphoreType.DMA((NE,)),
]


@jax.jit
def pallas_sequential_preLN__sliding_block_cached__glu_gated_swiglu__decode_kernel(
    A_x, A_k_cache, A_v_cache, A_wq, A_wo, B_x, B_w1, B_w3, B_w2,
):
    kt = jnp.swapaxes(A_k_cache, 2, 3).reshape(H, DH, SK)
    vt = jnp.swapaxes(A_v_cache, 2, 3).reshape(H, DH, SK)
    return pl.pallas_call(
        _kernel,
        in_specs=[pl.BlockSpec(memory_space=pl.ANY)] * 8,
        out_specs=pl.BlockSpec(memory_space=pltpu.VMEM),
        out_shape=jax.ShapeDtypeStruct((1, 1, D), jnp.bfloat16),
        scratch_shapes=_SCRATCH,
        compiler_params=pltpu.CompilerParams(vmem_limit_bytes=64 * 1024 * 1024),
    )(A_x, kt, vt, A_wq, A_wo, B_w1, B_w3, B_w2)
```
